```python
import os as _os
_os.environ.setdefault("JAX_PLATFORMS", "cpu")
import jax
import jax.numpy as jnp

def _softmax(x, axis=-1):
    return jax.nn.softmax(x, axis=axis)
def _gelu(x):
    return jax.nn.gelu(x, approximate=True)
def _silu(x):
    return jax.nn.silu(x)
def _sigmoid(x):
    return jax.nn.sigmoid(x)
def _layernorm(x, axis=-1, eps=1e-5):
    m = jnp.mean(x, axis=axis, keepdims=True)
    v = jnp.var(x, axis=axis, keepdims=True)
    return (x - m) / jnp.sqrt(v + eps)
def _scatter_add(tgt, idx, src, axis=0):
    return tgt.at[idx].add(src)
def _segment_sum(src, seg, n):
    return jax.ops.segment_sum(src, seg, n)
class _Rng:
    def __init__(self, key):
        self._k = key
    def _next(self):
        self._k, sub = jax.random.split(self._k)
        return sub
    def normal(self, shape):
        return jax.random.normal(self._next(), shape, dtype=jnp.bfloat16)
    def randint(self, lo, hi, shape):
        return jax.random.randint(self._next(), shape, lo, hi, dtype=jnp.int32)
    def uniform(self, shape, lo=0.0, hi=1.0):
        return jax.random.uniform(self._next(), shape, jnp.bfloat16, lo, hi)
    def permutation(self, n):
        return jax.random.permutation(self._next(), n)


kernel_name = 'standalone__gqa_block_cached__near_ridge'

def setup_inputs():
    _rng = _Rng(jax.random.key(int.from_bytes(__import__("os").urandom(4), "little")))
    _w = (lambda a: (lambda t: t.astype(jnp.bfloat16) if jnp.issubdtype(t.dtype, jnp.floating) else t)(jnp.asarray(a)))
    B, Sq, D = 8, 96, 640
    Hq, Hkv, Sk, Dh = 32, 32, 512, 128
    assert Hq % Hkv == 0, (Hq, Hkv)
    return {
        "x": _w((lambda *s: _rng.normal(s) * 0.2)(B, Sq, D)),
        "k_cache": _w((lambda *s: _rng.normal(s) * 3.2)(B, Hkv, Sk, Dh)),
        "v_cache": _w((lambda *s: _rng.normal(s) * 0.05)(B, Hkv, Sk, Dh)),
        "wq": _w((lambda *s: _rng.normal(s) * 0.2)(D, Hq * Dh) * (D ** -0.5)),
        "wo": _w((lambda *s: _rng.normal(s) * 0.05)(Hq * Dh, D) * ((Hq * Dh) ** -0.5)),
    }

def reference(x, k_cache, v_cache, wq, wo):
    B, Sq, D = x.shape
    Hq, Dh = 32, 128
    Hkv = k_cache.shape[1]
    rep = Hq // Hkv
    q = (lambda x, *d: x.transpose(*d))((x @ wq).reshape(B, Sq, Hq, Dh), 0, 2, 1, 3)
    k = jnp.repeat(k_cache, rep, axis=1)
    v = jnp.repeat(v_cache, rep, axis=1)
    scores = jnp.einsum("bhqd,bhkd->bhqk", q, k) * (Dh ** -0.5)
    p = _softmax(scores, axis=-1)
    o = jnp.einsum("bhqk,bhkd->bhqd", p, v)
    return (lambda x, *d: x.transpose(*d))(o, 0, 2, 1, 3).reshape(B, Sq, Hq * Dh) @ wo
```

```python
import functools

import jax
import jax.numpy as jnp
import jax.experimental.pallas as pl
import jax.experimental.pallas.tpu as pltpu


def _kernel(x_ref, k_ref, v_ref, wq_ref, wo_ref, out_ref, acc_ref, *, B, Sq, hb, scale):
    h = pl.program_id(0)
    nh = pl.num_programs(0)

    @pl.when(h == 0)
    def _():
        acc_ref[...] = jnp.zeros_like(acc_ref)

    x = x_ref[...]
    for j in range(hb):
        wq = wq_ref[:, j * 128:(j + 1) * 128]
        q = jnp.dot(x, wq, preferred_element_type=jnp.float32) * scale
        q = q.astype(jnp.bfloat16)
        outs = []
        for b in range(B):
            qb = q[b * Sq:(b + 1) * Sq]
            k = k_ref[b, j]
            v = v_ref[b, j]
            s = jax.lax.dot_general(qb, k, (((1,), (1,)), ((), ())),
                                    preferred_element_type=jnp.float32)
            m = jnp.max(s, axis=-1, keepdims=True)
            p = jnp.exp(s - m)
            l = jnp.sum(p, axis=-1, keepdims=True)
            o = jnp.dot(p.astype(jnp.bfloat16), v, preferred_element_type=jnp.float32)
            o = o / l
            outs.append(o.astype(jnp.bfloat16))
        o_all = jnp.concatenate(outs, axis=0)
        acc_ref[...] += jnp.dot(o_all, wo_ref[j * 128:(j + 1) * 128, :],
                                preferred_element_type=jnp.float32)

    @pl.when(h == nh - 1)
    def _():
        out_ref[...] = acc_ref[...].astype(out_ref.dtype)


@jax.jit
def pallas_standalone__gqa_block_cached__near_ridge_kernel(x, k_cache, v_cache, wq, wo):
    B, Sq, D = x.shape
    Hkv, Sk, Dh = k_cache.shape[1], k_cache.shape[2], k_cache.shape[3]
    Hq = wq.shape[1] // Dh
    assert Hq == Hkv
    hb = 1
    x2 = x.reshape(B * Sq, D)
    kern = functools.partial(_kernel, B=B, Sq=Sq, hb=hb, scale=Dh ** -0.5)
    out = pl.pallas_call(
        kern,
        grid=(Hq // hb,),
        in_specs=[
            pl.BlockSpec((B * Sq, D), lambda h: (0, 0)),
            pl.BlockSpec((B, hb, Sk, Dh), lambda h: (0, h, 0, 0)),
            pl.BlockSpec((B, hb, Sk, Dh), lambda h: (0, h, 0, 0)),
            pl.BlockSpec((D, hb * Dh), lambda h: (0, h)),
            pl.BlockSpec((hb * Dh, D), lambda h: (h, 0)),
        ],
        out_specs=pl.BlockSpec((B * Sq, D), lambda h: (0, 0)),
        out_shape=jax.ShapeDtypeStruct((B * Sq, D), x.dtype),
        scratch_shapes=[pltpu.VMEM((B * Sq, D), jnp.float32)],
        compiler_params=pltpu.CompilerParams(
            dimension_semantics=("arbitrary",),
            vmem_limit_bytes=64 * 1024 * 1024,
        ),
    )(x2, k_cache, v_cache, wq, wo)
    return out.reshape(B, Sq, D)
```

```python
import functools

import jax
import jax.numpy as jnp
import jax.experimental.pallas as pl
import jax.experimental.pallas.tpu as pltpu

_NUM_MXU = 4
_MXU_N = 128


def _kernel(x_hbm, k_hbm, v_hbm, wq_hbm, wo_hbm, out_hbm,
            x_buf, k_buf, v_buf, wq_buf, wo_buf, acc_ref, p_ref, l_ref, out_buf,
            k_sem, v_sem, wq_sem, wo_sem, x_sem, out_sem,
            *, B, Sq, H, rep, Dh, D, scale, n_out_parts):
    h = pl.program_id(0)
    slot = h % 2

    def k_copy(hh):
        return pltpu.make_async_copy(k_hbm.at[:, hh // rep], k_buf.at[hh % 2], k_sem.at[hh % 2])

    def v_copy(hh):
        return pltpu.make_async_copy(v_hbm.at[:, hh // rep], v_buf.at[hh % 2], v_sem.at[hh % 2])

    def wq_copy(hh):
        return pltpu.make_async_copy(wq_hbm.at[:, pl.ds(pl.multiple_of(hh * Dh, Dh), Dh)],
                                     wq_buf.at[hh % 2], wq_sem.at[hh % 2])

    def wo_copy(hh):
        return pltpu.make_async_copy(wo_hbm.at[pl.ds(pl.multiple_of(hh * Dh, Dh), Dh), :],
                                     wo_buf.at[hh % 2], wo_sem.at[hh % 2])

    b_part = B // n_out_parts
    m_part = b_part * Sq

    def out_copy(part):
        rows = slice(part * m_part, (part + 1) * m_part)
        return pltpu.make_async_copy(out_buf.at[rows], out_hbm.at[rows], out_sem.at[part])

    x_copy = pltpu.make_async_copy(x_hbm, x_buf, x_sem)

    def issue(hh):
        wq_copy(hh).start()
        k_copy(hh).start()
        wo_copy(hh).start()
        v_copy(hh).start()

    @pl.when(h == 0)
    def _():
        x_copy.start()
        issue(0)
        if H > 1:
            issue(1)
        acc_ref[...] = jnp.zeros_like(acc_ref)
        x_copy.wait()

    @pl.when(jnp.logical_and(h > 0, h + 1 < H))
    def _():
        issue(h + 1)

    wq_copy(h).wait()
    k_copy(h).wait()

    q = jnp.dot(x_buf[...], wq_buf[slot], preferred_element_type=jnp.float32) * scale
    q = q.astype(jnp.bfloat16)
    for b in range(B):
        r = slice(b * Sq, (b + 1) * Sq)
        s = jax.lax.dot_general(q[r], k_buf[slot, b], (((1,), (1,)), ((), ())),
                                preferred_element_type=jnp.float32)
        m = jnp.max(s, axis=-1, keepdims=True)
        p = jnp.exp(s - m)
        l_ref[r, :] = jnp.sum(p, axis=-1, keepdims=True)
        p_ref[r, :] = p.astype(p_ref.dtype)

    wo_copy(h).wait()
    v_copy(h).wait()

    wide = _NUM_MXU * _MXU_N
    d_main = (D // wide) * wide

    def phase1(b0, b1, dst):
        outs = []
        for b in range(b0, b1):
            r = slice(b * Sq, (b + 1) * Sq)
            o = jnp.dot(p_ref[r, :], v_buf[slot, b], preferred_element_type=jnp.float32)
            o = o / l_ref[r, :]
            outs.append(o.astype(jnp.bfloat16))
        o_all = outs[0] if len(outs) == 1 else jnp.concatenate(outs, axis=0)
        wo = wo_buf[slot]
        r0 = b0 * Sq
        mp = (b1 - b0) * Sq

        def proj(rows_src, rows_dst, cols):
            y = jnp.dot(o_all[rows_src], wo[:, cols], preferred_element_type=jnp.float32)
            dst[rows_dst, cols] = (acc_ref[rows_dst, cols] + y).astype(dst.dtype)

        if d_main:
            proj(slice(0, mp), slice(r0, r0 + mp), slice(0, d_main))
        if d_main < D:
            n_split = _NUM_MXU if mp % (8 * _NUM_MXU) == 0 else 1
            step = mp // n_split
            for c in range(n_split):
                proj(slice(c * step, (c + 1) * step),
                     slice(r0 + c * step, r0 + (c + 1) * step), slice(d_main, D))

    @pl.when(h < H - 1)
    def _():
        phase1(0, B, acc_ref)

    @pl.when(h == H - 1)
    def _():
        for part in range(n_out_parts):
            phase1(part * b_part, (part + 1) * b_part, out_buf)
            out_copy(part).start()
        for part in range(n_out_parts):
            out_copy(part).wait()


@jax.jit
def pallas_standalone__gqa_block_cached__near_ridge_kernel(
    x: jax.Array,
    k_cache: jax.Array,
    v_cache: jax.Array,
    wq: jax.Array,
    wo: jax.Array,
):
    B, Sq, D = x.shape
    Hkv, Sk, Dh = k_cache.shape[1], k_cache.shape[2], k_cache.shape[3]
    Hq = wq.shape[1] // Dh
    assert Hq % Hkv == 0
    rep = Hq // Hkv
    M = B * Sq
    n_out_parts = 4 if B % 4 == 0 else 1

    kern = functools.partial(_kernel, B=B, Sq=Sq, H=Hq, rep=rep, Dh=Dh, D=D,
                             scale=Dh ** -0.5, n_out_parts=n_out_parts)
    any_spec = pl.BlockSpec(memory_space=pl.ANY)
    out = pl.pallas_call(
        kern,
        grid=(Hq,),
        in_specs=[any_spec] * 5,
        out_specs=any_spec,
        out_shape=jax.ShapeDtypeStruct((M, D), x.dtype),
        scratch_shapes=[
            pltpu.VMEM((M, D), x.dtype),
            pltpu.VMEM((2, B, Sk, Dh), k_cache.dtype),
            pltpu.VMEM((2, B, Sk, Dh), v_cache.dtype),
            pltpu.VMEM((2, D, Dh), wq.dtype),
            pltpu.VMEM((2, Dh, D), wo.dtype),
            pltpu.VMEM((M, D), jnp.float32),
            pltpu.VMEM((M, Sk), jnp.bfloat16),
            pltpu.VMEM((M, 1), jnp.float32),
            pltpu.VMEM((M, D), x.dtype),
            pltpu.SemaphoreType.DMA((2,)),
            pltpu.SemaphoreType.DMA((2,)),
            pltpu.SemaphoreType.DMA((2,)),
            pltpu.SemaphoreType.DMA((2,)),
            pltpu.SemaphoreType.DMA,
            pltpu.SemaphoreType.DMA((n_out_parts,)),
        ],
        compiler_params=pltpu.CompilerParams(
            dimension_semantics=("arbitrary",),
            vmem_limit_bytes=64 * 1024 * 1024,
        ),
    )(x.reshape(M, D), k_cache, v_cache, wq, wo)
    return out.reshape(B, Sq, D)
```
